```python
import os as _os
_os.environ.setdefault('JAX_PLATFORMS', 'cpu')
import jax
import jax.numpy as jnp

def _softmax(x, axis=-1):
    return jax.nn.softmax(x, axis=axis)

def _gelu(x):
    return jax.nn.gelu(x, approximate=True)

def _silu(x):
    return jax.nn.silu(x)

def _sigmoid(x):
    return jax.nn.sigmoid(x)

def _layernorm(x, axis=-1, eps=1e-05):
    m = jnp.mean(x, axis=axis, keepdims=True)
    v = jnp.var(x, axis=axis, keepdims=True)
    return (x - m) / jnp.sqrt(v + eps)

def _scatter_add(tgt, idx, src, axis=0):
    return tgt.at[idx].add(src)

def _segment_sum(src, seg, n):
    return jax.ops.segment_sum(src, seg, n)

class _Rng:

    def __init__(self, key):
        self._k = key

    def _next(self):
        self._k, sub = jax.random.split(self._k)
        return sub

    def normal(self, shape):
        return jax.random.normal(self._next(), shape, dtype=jnp.bfloat16)

    def randint(self, lo, hi, shape):
        return jax.random.randint(self._next(), shape, lo, hi, dtype=jnp.int32)

    def uniform(self, shape, lo=0.0, hi=1.0):
        return jax.random.uniform(self._next(), shape, jnp.bfloat16, lo, hi)

    def permutation(self, n):
        return jax.random.permutation(self._next(), n)
kernel_name = 'standalone__conformer_conv_module__speech'

def setup_inputs():
    _rng = _Rng(jax.random.key(int.from_bytes(__import__("os").urandom(4), "little")))
    _w = lambda a: (lambda t: t.astype(jnp.bfloat16) if jnp.issubdtype(t.dtype, jnp.floating) else t)(jnp.asarray(a))
    B, T, D, K = (2, 16000, 256, 5)
    return {'x': _w((lambda *s: _rng.normal(s) * 0.2)(B, T, D)), 'w_pw1': _w((lambda *s: _rng.normal(s) * 0.2)(D, 2 * D)), 'dw': _w((lambda *s: _rng.normal(s) * 0.05)(K, D)), 'w_pw2': _w((lambda *s: _rng.normal(s) * 0.05)(D, D))}

def reference(x, w_pw1, dw, w_pw2):
    B, T, D = x.shape
    K = dw.shape[0]
    h = x @ w_pw1
    a, b = (h[..., :D].copy(), h[..., D:].copy())
    h = a * _sigmoid(b)
    pad = K // 2
    hp = jnp.pad(h, ((0, 0), (pad, pad), (0, 0)))
    out = jnp.zeros_like(h)
    for i in range(K):
        out = out + hp[:, i:i + T, :] * dw[i][None, None, :]
    return _silu(out) @ w_pw2
```

```python
import functools

import jax
import jax.numpy as jnp
import jax.experimental.pallas as pl
import jax.experimental.pallas.tpu as pltpu

HALO = 16


def _kernel(xp_ref, x_ref, xn_ref, w1_ref, dw_ref, w2_ref, o_ref, h_ref, *, tm, d, k):
    i = pl.program_id(1)
    n = pl.num_programs(1)
    pad = k // 2
    w1 = w1_ref[...]

    def glu(xv):
        h = jnp.dot(xv, w1, preferred_element_type=jnp.float32)
        return h[:, :d] * jax.nn.sigmoid(h[:, d:])

    hp = glu(xp_ref[0])
    hn = glu(xn_ref[0])
    h_ref[pl.ds(0, HALO), :] = jnp.where(i > 0, hp, 0.0)
    h_ref[pl.ds(HALO, tm), :] = glu(x_ref[0])
    h_ref[pl.ds(HALO + tm, HALO), :] = jnp.where(i < n - 1, hn, 0.0)

    dw = dw_ref[...].astype(jnp.float32)
    acc = h_ref[pl.ds(HALO - pad, tm), :] * dw[0:1, :]
    for j in range(1, k):
        acc = acc + h_ref[pl.ds(HALO - pad + j, tm), :] * dw[j:j + 1, :]
    g = acc * jax.nn.sigmoid(acc)
    o_ref[0] = jnp.dot(g.astype(jnp.bfloat16), w2_ref[...],
                       preferred_element_type=jnp.float32).astype(o_ref.dtype)


@jax.jit
def pallas_standalone__conformer_conv_module__speech_kernel(
    x: jax.Array,
    w_pw1: jax.Array,
    dw: jax.Array,
    w_pw2: jax.Array,
):
    B, T, D = x.shape
    K = dw.shape[0]
    tm = 1600
    assert T % tm == 0 and tm % HALO == 0
    nt = T // tm
    r = tm // HALO
    nh = T // HALO

    kernel = functools.partial(_kernel, tm=tm, d=D, k=K)
    return pl.pallas_call(
        kernel,
        grid=(B, nt),
        in_specs=[
            pl.BlockSpec((1, HALO, D), lambda b, i: (b, jnp.maximum(i * r - 1, 0), 0)),
            pl.BlockSpec((1, tm, D), lambda b, i: (b, i, 0)),
            pl.BlockSpec((1, HALO, D), lambda b, i: (b, jnp.minimum((i + 1) * r, nh - 1), 0)),
            pl.BlockSpec((D, 2 * D), lambda b, i: (0, 0)),
            pl.BlockSpec((K, D), lambda b, i: (0, 0)),
            pl.BlockSpec((D, D), lambda b, i: (0, 0)),
        ],
        out_specs=pl.BlockSpec((1, tm, D), lambda b, i: (b, i, 0)),
        out_shape=jax.ShapeDtypeStruct((B, T, D), x.dtype),
        scratch_shapes=[pltpu.VMEM((tm + 2 * HALO, D), jnp.float32)],
        compiler_params=pltpu.CompilerParams(
            dimension_semantics=("parallel", "arbitrary"),
            vmem_limit_bytes=64 * 1024 * 1024,
        ),
    )(x, x, x, w_pw1, dw, w_pw2)
```

```python
import functools

import jax
import jax.numpy as jnp
from jax import lax
import jax.experimental.pallas as pl
import jax.experimental.pallas.tpu as pltpu

HALO = 16
LANE = 128
TM = 8000
MINIS = (400, 1200, 2400, 4000)
SEGS = (4000, 2400, 1200, 400)
OUT_MAX = 1200


def _kernel(x_hbm, w1_hbm, dw_hbm, w2_hbm, o_hbm,
            xbuf, obuf, w1buf, w1s, dwbuf, w2buf, hcar, isem, osem, wsem,
            *, tm, minis, segs, t_len, d, k):
    rows = x_hbm.shape[0]
    n = rows // tm
    cpb = t_len // tm
    pad = k // 2
    nc = d // LANE

    def al(r):
        return r if isinstance(r, int) else pl.multiple_of(r, HALO)

    def seg_desc(start, size, s):
        return pltpu.make_async_copy(x_hbm.at[pl.ds(al(start), size)],
                                     xbuf.at[pl.ds(al(start + HALO), size)], isem.at[s])

    def seg_start(start, size, s):
        if size >= 1600:
            h = (size // 2) // HALO * HALO
            seg_desc(start, h, s).start()
            seg_desc(start + h, size - h, s).start()
        else:
            seg_desc(start, size, s).start()

    def seg_wait(start, size, s):
        seg_desc(start, size, s).wait()

    def chunk_args(j, last):
        return (j * tm + HALO, tm - HALO if last else tm, j % 2)

    w1c = pltpu.make_async_copy(w1_hbm, w1buf, wsem.at[0])
    dwc_ = pltpu.make_async_copy(dw_hbm, dwbuf, wsem.at[1])
    w2c = pltpu.make_async_copy(w2_hbm, w2buf, wsem.at[2])

    mini_starts = [sum(minis[:i]) for i in range(len(minis))]
    mini_args = []
    for i, (s, m) in enumerate(zip(mini_starts, minis)):
        mini_args.append((0, m + HALO, 2) if i == 0 else (s + HALO, m, 2 + i))

    w1c.start()
    seg_start(*mini_args[0])
    dwc_.start()
    w2c.start()
    xbuf[pl.ds(0, HALO), :] = jnp.zeros((HALO, d), xbuf.dtype)
    xbuf[pl.ds(rows + HALO, HALO), :] = jnp.zeros((HALO, d), xbuf.dtype)
    w1c.wait()
    seg_start(*mini_args[1])
    for c in range(nc):
        w1s[:, pl.ds(2 * c * LANE, LANE)] = w1buf[:, pl.ds(c * LANE, LANE)]
        wb = w1buf[:, pl.ds(d + c * LANE, LANE)].astype(jnp.float32) * 0.5
        w1s[:, pl.ds((2 * c + 1) * LANE, LANE)] = wb.astype(w1s.dtype)
    dwc_.wait()
    w2c.wait()

    def process(r0, size, keep_left, keep_right, segs, first_unit):
        dws = dwbuf[...].astype(jnp.float32) * 0.25
        w2 = w2buf[...]
        tails = [None] * nc
        off = 0
        ns = len(segs)
        for si, sz in enumerate(segs):
            first, last = si == 0, si == ns - 1
            fresh = first and first_unit
            lo = off if fresh else off + 2 * HALO
            hi = off + sz + 2 * HALO
            m = hi - lo
            xx = xbuf[pl.ds(al(r0 + lo), m), :]
            gs = []
            for c in range(nc):
                hh = jnp.dot(xx, w1s[:, pl.ds(2 * c * LANE, 2 * LANE)],
                             preferred_element_type=jnp.float32)
                a = hh[:, :LANE]
                h2 = a + a * jnp.tanh(hh[:, LANE:])
                parts = []
                if fresh:
                    parts.append(jnp.where(keep_left, h2[:HALO], 0.0))
                    body_lo = HALO
                elif first:
                    t = hcar[c]
                    parts.append(jnp.where(keep_left, t[:HALO], 0.0))
                    parts.append(t[HALO:])
                    body_lo = 0
                else:
                    parts.append(tails[c])
                    body_lo = 0
                if last:
                    hcar[c] = h2[m - 2 * HALO:]
                    parts.append(h2[body_lo:m - HALO])
                    parts.append(jnp.where(keep_right, h2[m - HALO:], 0.0))
                else:
                    parts.append(h2[body_lo:])
                    tails[c] = h2[m - 2 * HALO:]
                h2 = jnp.concatenate(parts, axis=0)
                dwc = dws[:, c * LANE:(c + 1) * LANE]
                acc = h2[HALO:HALO + sz] * dwc[pad:pad + 1, :]
                for jj in range(k):
                    if jj == pad:
                        continue
                    o = HALO - pad + jj
                    acc = acc + h2[o:o + sz] * dwc[jj:jj + 1, :]
                g = acc + acc * jnp.tanh(acc)
                gs.append(g.astype(jnp.bfloat16))
            g = jnp.concatenate(gs, axis=1)
            npieces = -(-sz // OUT_MAX)
            ps = sz // npieces // HALO * HALO
            po = 0
            for pi in range(npieces):
                pz = ps if pi < npieces - 1 else sz - po
                o = jnp.dot(g[po:po + pz], w2, preferred_element_type=jnp.float32)
                r = al(r0 + off + po)
                obuf[pl.ds(r, pz), :] = o.astype(obuf.dtype)
                pltpu.make_async_copy(obuf.at[pl.ds(r, pz)], o_hbm.at[pl.ds(r, pz)],
                                      osem.at[0]).start()
                po += pz
            off += sz

    nm = len(minis)
    for i, (s, m) in enumerate(zip(mini_starts, minis)):
        seg_wait(*mini_args[i])
        if i + 2 < nm:
            seg_start(*mini_args[i + 2])
        if i + 2 == nm:
            seg_start(*chunk_args(1, n == 2))
        process(s, m, s % t_len != 0, (s + m) % t_len != 0, (m,), i == 0)

    def body(j, carry):
        @pl.when(j < n - 1)
        def _():
            seg_wait(*chunk_args(j, False))

        @pl.when(j == n - 1)
        def _():
            seg_wait(*chunk_args(j, True))

        @pl.when(j + 1 < n - 1)
        def _():
            seg_start(*chunk_args(j + 1, False))

        @pl.when(j + 1 == n - 1)
        def _():
            seg_start(*chunk_args(j + 1, True))

        jb = j % cpb
        process(j * tm, tm, jb > 0, jb < cpb - 1, segs, False)
        return carry

    lax.fori_loop(1, n, body, 0)
    pltpu.make_async_copy(obuf, o_hbm, osem.at[0]).wait()


@jax.jit
def pallas_standalone__conformer_conv_module__speech_kernel(
    x: jax.Array,
    w_pw1: jax.Array,
    dw: jax.Array,
    w_pw2: jax.Array,
):
    B, T, D = x.shape
    K = dw.shape[0]
    tm = TM
    assert T % tm == 0 and sum(MINIS) == tm and len(MINIS) >= 2 and sum(SEGS) == tm
    R = B * T

    kernel = functools.partial(_kernel, tm=tm, minis=MINIS, segs=SEGS,
                               t_len=T, d=D, k=K)
    anyspec = pl.BlockSpec(memory_space=pl.ANY)
    out = pl.pallas_call(
        kernel,
        in_specs=[anyspec, anyspec, anyspec, anyspec],
        out_specs=anyspec,
        out_shape=jax.ShapeDtypeStruct((R, D), x.dtype),
        scratch_shapes=[
            pltpu.VMEM((R + 2 * HALO, D), x.dtype),
            pltpu.VMEM((R, D), x.dtype),
            pltpu.VMEM((D, 2 * D), w_pw1.dtype),
            pltpu.VMEM((D, 2 * D), w_pw1.dtype),
            pltpu.VMEM((K, D), dw.dtype),
            pltpu.VMEM((D, D), w_pw2.dtype),
            pltpu.VMEM((D // LANE, 2 * HALO, LANE), jnp.float32),
            pltpu.SemaphoreType.DMA((2 + len(MINIS),)),
            pltpu.SemaphoreType.DMA((1,)),
            pltpu.SemaphoreType.DMA((3,)),
        ],
        compiler_params=pltpu.CompilerParams(
            vmem_limit_bytes=100 * 1024 * 1024,
            disable_bounds_checks=True,
        ),
    )(x.reshape(R, D), w_pw1, dw, w_pw2)
    return out.reshape(B, T, D)
```

```python
import functools

import jax
import jax.numpy as jnp
from jax import lax
import jax.experimental.pallas as pl
import jax.experimental.pallas.tpu as pltpu

HALO = 16
LANE = 128
TM = 8000
MINIS = (320, 1120, 2560, 4000)
SEGS = (4000, 2400, 1344, 256)
OUT_MAX = 1200


def _kernel(x_hbm, w1_hbm, dw_hbm, w2_hbm, o_hbm,
            xbuf, obuf, w1buf, w1s, dwbuf, w2buf, hcar, isem, osem, wsem,
            *, tm, minis, segs, t_len, d, k):
    rows = x_hbm.shape[0]
    n = rows // tm
    cpb = t_len // tm
    pad = k // 2
    nc = d // LANE

    def al(r):
        return r if isinstance(r, int) else pl.multiple_of(r, HALO)

    def seg_desc(start, size, s):
        return pltpu.make_async_copy(x_hbm.at[pl.ds(al(start), size)],
                                     xbuf.at[pl.ds(al(start + HALO), size)], isem.at[s])

    def seg_start(start, size, s):
        if size >= 1600:
            h = (size // 2) // HALO * HALO
            seg_desc(start, h, s).start()
            seg_desc(start + h, size - h, s).start()
        else:
            seg_desc(start, size, s).start()

    def seg_wait(start, size, s):
        seg_desc(start, size, s).wait()

    def chunk_args(j, last):
        return (j * tm + HALO, tm - HALO if last else tm, j % 2)

    w1c = pltpu.make_async_copy(w1_hbm, w1buf, wsem.at[0])
    dwc_ = pltpu.make_async_copy(dw_hbm, dwbuf, wsem.at[1])
    w2c = pltpu.make_async_copy(w2_hbm, w2buf, wsem.at[2])

    mini_starts = [sum(minis[:i]) for i in range(len(minis))]
    mini_args = []
    for i, (s, m) in enumerate(zip(mini_starts, minis)):
        mini_args.append((0, m + HALO, 2) if i == 0 else (s + HALO, m, 2 + i))

    w1c.start()
    seg_start(*mini_args[0])
    dwc_.start()
    w2c.start()
    xbuf[pl.ds(0, HALO), :] = jnp.zeros((HALO, d), xbuf.dtype)
    xbuf[pl.ds(rows + HALO, HALO), :] = jnp.zeros((HALO, d), xbuf.dtype)
    w1c.wait()
    seg_start(*mini_args[1])
    for c in range(nc):
        w1s[:, pl.ds(2 * c * LANE, LANE)] = w1buf[:, pl.ds(c * LANE, LANE)]
        wb = w1buf[:, pl.ds(d + c * LANE, LANE)].astype(jnp.float32) * 0.5
        w1s[:, pl.ds((2 * c + 1) * LANE, LANE)] = wb.astype(w1s.dtype)
    dwc_.wait()
    w2c.wait()

    def process(r0, size, keep_left, keep_right, segs, first_unit):
        dws = dwbuf[...].astype(jnp.float32) * 0.25
        w2 = w2buf[...]
        tails = [None] * nc
        off = 0
        ns = len(segs)
        for si, sz in enumerate(segs):
            first, last = si == 0, si == ns - 1
            fresh = first and first_unit
            lo = off if fresh else off + 2 * HALO
            hi = off + sz + 2 * HALO
            m = hi - lo
            xx = xbuf[pl.ds(al(r0 + lo), m), :]
            gs = []
            for c in range(nc):
                hh = jnp.dot(xx, w1s[:, pl.ds(2 * c * LANE, 2 * LANE)],
                             preferred_element_type=jnp.float32)
                a = hh[:, :LANE]
                h2 = a + a * jnp.tanh(hh[:, LANE:])
                parts = []
                if fresh:
                    parts.append(jnp.where(keep_left, h2[:HALO], 0.0))
                    body_lo = HALO
                elif first:
                    t = hcar[c]
                    parts.append(jnp.where(keep_left, t[:HALO], 0.0))
                    parts.append(t[HALO:])
                    body_lo = 0
                else:
                    parts.append(tails[c])
                    body_lo = 0
                if last:
                    hcar[c] = h2[m - 2 * HALO:]
                    parts.append(h2[body_lo:m - HALO])
                    parts.append(jnp.where(keep_right, h2[m - HALO:], 0.0))
                else:
                    parts.append(h2[body_lo:])
                    tails[c] = h2[m - 2 * HALO:]
                h2 = jnp.concatenate(parts, axis=0)
                dwc = dws[:, c * LANE:(c + 1) * LANE]
                acc = h2[HALO:HALO + sz] * dwc[pad:pad + 1, :]
                for jj in range(k):
                    if jj == pad:
                        continue
                    o = HALO - pad + jj
                    acc = acc + h2[o:o + sz] * dwc[jj:jj + 1, :]
                g = acc + acc * jnp.tanh(acc)
                gs.append(g.astype(jnp.bfloat16))
            g = jnp.concatenate(gs, axis=1)
            npieces = -(-sz // OUT_MAX)
            ps = sz // npieces // HALO * HALO
            po = 0
            for pi in range(npieces):
                pz = ps if pi < npieces - 1 else sz - po
                o = jnp.dot(g[po:po + pz], w2, preferred_element_type=jnp.float32)
                r = al(r0 + off + po)
                obuf[pl.ds(r, pz), :] = o.astype(obuf.dtype)
                pltpu.make_async_copy(obuf.at[pl.ds(r, pz)], o_hbm.at[pl.ds(r, pz)],
                                      osem.at[0]).start()
                po += pz
            off += sz

    nm = len(minis)
    for i, (s, m) in enumerate(zip(mini_starts, minis)):
        seg_wait(*mini_args[i])
        if i + 2 < nm:
            seg_start(*mini_args[i + 2])
        if i + 2 == nm:
            seg_start(*chunk_args(1, n == 2))
        process(s, m, s % t_len != 0, (s + m) % t_len != 0, (m,), i == 0)

    def body(j, carry):
        @pl.when(j < n - 1)
        def _():
            seg_wait(*chunk_args(j, False))

        @pl.when(j == n - 1)
        def _():
            seg_wait(*chunk_args(j, True))

        @pl.when(j + 1 < n - 1)
        def _():
            seg_start(*chunk_args(j + 1, False))

        @pl.when(j + 1 == n - 1)
        def _():
            seg_start(*chunk_args(j + 1, True))

        jb = j % cpb
        process(j * tm, tm, jb > 0, jb < cpb - 1, segs, False)
        return carry

    lax.fori_loop(1, n, body, 0)
    pltpu.make_async_copy(obuf, o_hbm, osem.at[0]).wait()


@jax.jit
def pallas_standalone__conformer_conv_module__speech_kernel(
    x: jax.Array,
    w_pw1: jax.Array,
    dw: jax.Array,
    w_pw2: jax.Array,
):
    B, T, D = x.shape
    K = dw.shape[0]
    tm = TM
    R = B * T
    assert T % tm == 0 and R // tm >= 2 and D % LANE == 0 and K // 2 <= HALO
    assert sum(MINIS) == tm and len(MINIS) >= 2 and sum(SEGS) == tm

    kernel = functools.partial(_kernel, tm=tm, minis=MINIS, segs=SEGS,
                               t_len=T, d=D, k=K)
    anyspec = pl.BlockSpec(memory_space=pl.ANY)
    out = pl.pallas_call(
        kernel,
        in_specs=[anyspec, anyspec, anyspec, anyspec],
        out_specs=anyspec,
        out_shape=jax.ShapeDtypeStruct((R, D), x.dtype),
        scratch_shapes=[
            pltpu.VMEM((R + 2 * HALO, D), x.dtype),
            pltpu.VMEM((R, D), x.dtype),
            pltpu.VMEM((D, 2 * D), w_pw1.dtype),
            pltpu.VMEM((D, 2 * D), w_pw1.dtype),
            pltpu.VMEM((K, D), dw.dtype),
            pltpu.VMEM((D, D), w_pw2.dtype),
            pltpu.VMEM((D // LANE, 2 * HALO, LANE), jnp.float32),
            pltpu.SemaphoreType.DMA((2 + len(MINIS),)),
            pltpu.SemaphoreType.DMA((1,)),
            pltpu.SemaphoreType.DMA((3,)),
        ],
        compiler_params=pltpu.CompilerParams(
            vmem_limit_bytes=100 * 1024 * 1024,
            disable_bounds_checks=True,
        ),
    )(x.reshape(R, D), w_pw1, dw, w_pw2)
    return out.reshape(B, T, D)
```
